```python
import jax
import jax.numpy as jnp

def _softmax(x, axis=-1):
    return jax.nn.softmax(x, axis=axis)
def _gelu(x):
    return jax.nn.gelu(x, approximate=True)
def _silu(x):
    return jax.nn.silu(x)
def _sigmoid(x):
    return jax.nn.sigmoid(x)
def _layernorm(x, axis=-1, eps=1e-5):
    m = jnp.mean(x, axis=axis, keepdims=True)
    v = jnp.var(x, axis=axis, keepdims=True)
    return (x - m) / jnp.sqrt(v + eps)
def _scatter_add(tgt, idx, src, axis=0):
    return tgt.at[idx].add(src)
def _segment_sum(src, seg, n):
    return jax.ops.segment_sum(src, seg, n)
class _Rng:
    def __init__(self, key):
        self._k = key
    def _next(self):
        self._k, sub = jax.random.split(self._k)
        return sub
    def normal(self, shape):
        return jax.random.normal(self._next(), shape, dtype=jnp.bfloat16)
    def randint(self, lo, hi, shape):
        return jax.random.randint(self._next(), shape, lo, hi, dtype=jnp.int32)
    def uniform(self, shape, lo=0.0, hi=1.0):
        return jax.random.uniform(self._next(), shape, jnp.bfloat16, lo, hi)
    def permutation(self, n):
        return jax.random.permutation(self._next(), n)


kernel_name = 'recurrent_scan__sliding_block_cached__glu_gated_swiglu__decode'

def setup_inputs():
    _rng = _Rng(jax.random.key(int.from_bytes(__import__("os").urandom(4), "little")))
    _w = (lambda a: (lambda t: t.astype(jnp.bfloat16) if jnp.issubdtype(t.dtype, jnp.floating) else t)(jnp.asarray(a)))
    def _A_setup():
        B, Sq, D = 1, 1, 640
        Hq, Hkv, Sk, Dh = 32, 32, 32768, 192
        assert Hq % Hkv == 0, (Hq, Hkv)
        return {
            "x": _w((lambda *s: _rng.normal(s) * 0.05)(B, Sq, D)),
            "k_cache": _w((lambda *s: _rng.normal(s) * 0.05)(B, Hkv, Sk, Dh)),
            "v_cache": _w((lambda *s: _rng.normal(s) * 0.05)(B, Hkv, Sk, Dh)),
            "wq": _w((lambda *s: _rng.normal(s) * 0.05)(D, Hq * Dh) * (D ** -0.5)),
            "wo": _w((lambda *s: _rng.normal(s) * 0.05)(Hq * Dh, D) * ((Hq * Dh) ** -0.5)),
        }
    _A_in = _A_setup()

    def _B_setup():
        B, S, D, F = 1, 1, 640, 1536
        return {
            "x": _w((lambda *s: _rng.normal(s) * 0.05)(B, S, D)),
            "w1": _w((lambda *s: _rng.normal(s) * 0.05)(D, F) * (2.0 / D) ** 0.5),
            "w3": _w((lambda *s: _rng.normal(s) * 0.05)(D, F) * (2.0 / D) ** 0.5),
            "w2": _w((lambda *s: _rng.normal(s) * 0.05)(F, D) * (2.0 / F) ** 0.5),
        }
    _B_in = _B_setup()

    return {
        "A_x": _A_in["x"],
        "A_k_cache": _A_in["k_cache"],
        "A_v_cache": _A_in["v_cache"],
        "A_wq": _A_in["wq"],
        "A_wo": _A_in["wo"],
        "B_x": _B_in["x"],
        "B_w1": _B_in["w1"],
        "B_w3": _B_in["w3"],
        "B_w2": _B_in["w2"],
    }

def reference(A_x, A_k_cache, A_v_cache, A_wq, A_wo, B_x, B_w1, B_w3, B_w2):
    def _A_ref(x, k_cache, v_cache, wq, wo):
        B, Sq, D = x.shape
        Hq, Dh = 32, 192
        Hkv, Sk = k_cache.shape[1], k_cache.shape[2]
        W = min(4096, max(256, Sk // 4))
        rep = Hq // Hkv
        q = (lambda x, *d: x.transpose(*d))((x @ wq).reshape(B, Sq, Hq, Dh), 0, 2, 1, 3)
        k = jnp.repeat(k_cache[:, :, Sk - W:, :], rep, axis=1)
        v = jnp.repeat(v_cache[:, :, Sk - W:, :], rep, axis=1)
        scores = jnp.einsum("bhqd,bhkd->bhqk", q, k) * (Dh ** -0.5)
        p = _softmax(scores, axis=-1)
        o = jnp.einsum("bhqk,bhkd->bhqd", p, v)
        return (lambda x, *d: x.transpose(*d))(o, 0, 2, 1, 3).reshape(B, Sq, Hq * Dh) @ wo

    def _B_ref(x, w1, w3, w2):
        gate = jnp.einsum("bsd,df->bsf", x, w1)
        up = jnp.einsum("bsd,df->bsf", x, w3)
        h = _silu(gate) * up
        out = jnp.einsum("bsf,fd->bsd", h, w2)
        return out

    x = A_x
    xn = _layernorm(x, axis=-1)
    s = _A_ref(xn, A_k_cache, A_v_cache, A_wq, A_wo)
    g = _silu(_B_ref(xn, B_w1, B_w3, B_w2))
    return x + s * g
```

```python
import jax
import jax.numpy as jnp
import jax.experimental.pallas as pl
import jax.experimental.pallas.tpu as pltpu

_HQ, _DH = 32, 192
_LN_EPS = 1e-5
_LANES = 128
_SUB = 8

_KV_COLS = 2048
_WD_ROWS = 24
_WO_STAGE = 768
_SLAB = 256


def _silu(v):
    return v * (1.0 / (1.0 + jnp.exp(-v)))


def _start_all(copies):
    for i, cp in enumerate(copies):
        cp.start(priority=i % 2)


def _wait_filled(buf, sem):
    pltpu.make_async_copy(buf, buf, sem).wait()


def _kernel(x_hbm, kt_hbm, vt_hbm, wq_hbm, wo_hbm, w1_hbm, w3_hbm, w2_hbm, out_ref,
            x_vm, k_vm, v_vm, wq_vm, wo_vm, w1_vm, w3_vm, w2_vm,
            q_col, o_col, p_vm, x_sem, kv_sem, wq_sem, ff_sem, wo_sem):
    f32, bf16 = jnp.float32, jnp.bfloat16
    d_model = x_vm.shape[1]
    d_ff = w2_vm.shape[0]
    win = k_vm.shape[2]
    win0 = kt_hbm.shape[3] - win
    n_qblk = wq_vm.shape[1] // _KV_COLS
    n_wo = wo_vm.shape[0] // _WO_STAGE

    def start_kv(src, dst, sem, head, slot):
        _start_all([
            pltpu.make_async_copy(
                src.at[0, head, pl.ds(r, _SUB), pl.ds(win0 + c, _KV_COLS)],
                dst.at[slot, pl.ds(r, _SUB), pl.ds(c, _KV_COLS)],
                sem)
            for c in range(0, win, _KV_COLS) for r in range(0, _DH, _SUB)])

    def start_k(head):
        start_kv(kt_hbm, k_vm, kv_sem.at[0, head % 2], head, head % 2)

    def start_v(head):
        start_kv(vt_hbm, v_vm, kv_sem.at[1, head % 2], head, head % 2)

    def start_wq(blk):
        cols = pl.ds(blk * _KV_COLS, _KV_COLS)
        _start_all([
            pltpu.make_async_copy(wq_hbm.at[pl.ds(r, _SUB), cols],
                                  wq_vm.at[pl.ds(r, _SUB), cols], wq_sem.at[blk])
            for r in range(0, d_model, _SUB)])

    def start_rows(src, dst, sem, row0, n_rows, piece):
        _start_all([
            pltpu.make_async_copy(src.at[pl.ds(row0 + r, piece), :],
                                  dst.at[pl.ds(row0 + r, piece), :], sem)
            for r in range(0, n_rows, piece)])

    def start_wo(stage):
        start_rows(wo_hbm, wo_vm, wo_sem.at[stage], stage * _WO_STAGE, _WO_STAGE, _WD_ROWS)

    x_copy = pltpu.make_async_copy(x_hbm, x_vm, x_sem)
    x_copy.start()
    start_wq(0)
    x_copy.wait()
    x = x_vm[...].astype(f32)
    mean = jnp.mean(x, axis=-1, keepdims=True)
    xc = x - mean
    var = jnp.mean(xc * xc, axis=-1, keepdims=True)
    xn = xc / jnp.sqrt(var + _LN_EPS)
    xn8 = jnp.broadcast_to(xn, (_SUB, d_model)).astype(bf16)

    def project_q(blk):
        cols = pl.ds(blk * _KV_COLS, _KV_COLS)
        _wait_filled(wq_vm.at[:, cols], wq_sem.at[blk])
        q = jnp.dot(xn8, wq_vm[:, cols], preferred_element_type=f32) * (_DH ** -0.5)
        for c in range(0, _KV_COLS, _LANES):
            tile = jnp.broadcast_to(q[0:1, c:c + _LANES], (_LANES, _LANES))
            q_col[pl.ds(blk * _KV_COLS + c, _LANES), :] = tile.T

    upcoming = [lambda b=b: start_wq(b) for b in range(1, n_qblk)]
    upcoming += [
        lambda: start_rows(w1_hbm, w1_vm, ff_sem.at[0], 0, d_model, _SUB),
        lambda: start_rows(w3_hbm, w3_vm, ff_sem.at[1], 0, d_model, _SUB),
        lambda: start_rows(w2_hbm, w2_vm, ff_sem.at[2], 0, d_ff, _WD_ROWS),
        lambda: start_k(0),
        lambda: start_v(0),
    ]
    for blk in range(n_qblk):
        upcoming.pop(0)()
        project_q(blk)

    upcoming.pop(0)()
    _wait_filled(w1_vm, ff_sem.at[0])
    gate = jnp.dot(xn8, w1_vm[...], preferred_element_type=f32)
    upcoming.pop(0)()
    _wait_filled(w3_vm, ff_sem.at[1])
    up = jnp.dot(xn8, w3_vm[...], preferred_element_type=f32)
    hidden = (_silu(gate) * up).astype(bf16)
    upcoming.pop(0)()
    _wait_filled(w2_vm, ff_sem.at[2])
    g = _silu(jnp.dot(hidden, w2_vm[...], preferred_element_type=f32))[0:1, :]
    upcoming.pop(0)()

    def softmax_numerator(head):
        slot = head % 2
        _wait_filled(k_vm.at[slot], kv_sem.at[0, slot])
        q = q_col[pl.ds(pl.multiple_of(head * _DH, _SUB), _DH), :]
        q = jnp.concatenate([q] * (_SLAB // _LANES), axis=1)
        run_max = None
        for c in range(0, win, _SLAB):
            k = k_vm[slot, :, c:c + _SLAB].astype(f32)
            s = jnp.broadcast_to(jnp.sum(k * q, axis=0, keepdims=True), (_SUB, _SLAB))
            p_vm[:, c:c + _SLAB] = s
            run_max = s if run_max is None else jnp.maximum(run_max, s)
        row_max = jnp.max(run_max, axis=1, keepdims=True)
        total = None
        for c in range(0, win, _SLAB):
            p = jnp.exp(p_vm[:, c:c + _SLAB] - row_max)
            p_vm[:, c:c + _SLAB] = p
            total = p if total is None else total + p
        return jnp.sum(total, axis=1, keepdims=True)

    def weighted_values(head, denom):
        slot = head % 2
        _wait_filled(v_vm.at[slot], kv_sem.at[1, slot])
        acc = None
        for c in range(0, win, _SLAB):
            v = v_vm[slot, :, c:c + _SLAB].astype(f32)
            for t in range(0, _SLAB, _LANES):
                p = p_vm[:, c + t:c + t + _LANES]
                term = v[:, t:t + _LANES] * jnp.concatenate([p] * (_DH // _SUB), axis=0)
                acc = term if acc is None else acc + term
        o = jnp.sum(acc, axis=1, keepdims=True) / denom[0:1, :]
        o_col[pl.ds(pl.multiple_of(head * _DH, _SUB), _DH), :] = (
            jnp.broadcast_to(o, (_DH, _LANES)))

    def head_step(head, carry):
        start_k(head + 1)
        denom = softmax_numerator(head)
        start_v(head + 1)
        weighted_values(head, denom)
        return carry

    jax.lax.fori_loop(0, _HQ - 1, head_step, None)

    start_wo(0)
    denom = softmax_numerator(_HQ - 1)
    start_wo(1)
    weighted_values(_HQ - 1, denom)

    acc = jnp.zeros((_SUB, d_model), f32)
    for stage in range(n_wo):
        if stage + 2 < n_wo:
            start_wo(stage + 2)
        rows = pl.ds(stage * _WO_STAGE, _WO_STAGE)
        _wait_filled(wo_vm.at[rows, :], wo_sem.at[stage])
        for r in range(stage * _WO_STAGE, (stage + 1) * _WO_STAGE, _DH):
            w = wo_vm[r:r + _DH, :].astype(f32)
            o = jnp.concatenate([o_col[r:r + _DH, :]] * (d_model // _LANES), axis=1)
            acc = acc + jnp.sum((w * o).reshape(_DH // _SUB, _SUB, d_model), axis=0)
    s = jnp.sum(acc, axis=0, keepdims=True)
    out_ref[...] = (x + s * g).astype(out_ref.dtype)


@jax.jit
def pallas_recurrent_scan__sliding_block_cached__glu_gated_swiglu__decode_kernel(
    A_x: jax.Array,
    A_k_cache: jax.Array,
    A_v_cache: jax.Array,
    A_wq: jax.Array,
    A_wo: jax.Array,
    B_x: jax.Array,
    B_w1: jax.Array,
    B_w3: jax.Array,
    B_w2: jax.Array,
):
    del B_x
    batch, seq, d_model = A_x.shape
    _, n_kv, s_k, d_head = A_k_cache.shape
    assert (batch, seq, n_kv, d_head) == (1, 1, _HQ, _DH)
    win = min(4096, max(256, s_k // 4))
    assert win % _KV_COLS == 0 and A_wq.shape[1] % _KV_COLS == 0
    assert A_wo.shape[0] % _WO_STAGE == 0 and B_w2.shape[0] % _WD_ROWS == 0

    kt = jnp.swapaxes(A_k_cache, 2, 3)
    vt = jnp.swapaxes(A_v_cache, 2, 3)

    f32 = jnp.float32
    hbm = pl.BlockSpec(memory_space=pltpu.HBM)
    out = pl.pallas_call(
        _kernel,
        out_shape=jax.ShapeDtypeStruct((1, d_model), A_x.dtype),
        in_specs=[hbm] * 8,
        out_specs=pl.BlockSpec(memory_space=pltpu.VMEM),
        scratch_shapes=[
            pltpu.VMEM((1, d_model), A_x.dtype),
            pltpu.VMEM((2, _DH, win), kt.dtype),
            pltpu.VMEM((2, _DH, win), vt.dtype),
            pltpu.VMEM(A_wq.shape, A_wq.dtype),
            pltpu.VMEM(A_wo.shape, A_wo.dtype),
            pltpu.VMEM(B_w1.shape, B_w1.dtype),
            pltpu.VMEM(B_w3.shape, B_w3.dtype),
            pltpu.VMEM(B_w2.shape, B_w2.dtype),
            pltpu.VMEM((_HQ * _DH, _LANES), f32),
            pltpu.VMEM((_HQ * _DH, _LANES), f32),
            pltpu.VMEM((_SUB, win), f32),
            pltpu.SemaphoreType.DMA(()),
            pltpu.SemaphoreType.DMA((2, 2)),
            pltpu.SemaphoreType.DMA((A_wq.shape[1] // _KV_COLS,)),
            pltpu.SemaphoreType.DMA((3,)),
            pltpu.SemaphoreType.DMA((A_wo.shape[0] // _WO_STAGE,)),
        ],
        compiler_params=pltpu.CompilerParams(vmem_limit_bytes=64 * 1024 * 1024),
    )(A_x.reshape(1, d_model), kt, vt, A_wq, A_wo, B_w1, B_w3, B_w2)
    return out.reshape(A_x.shape)
```

```python
import jax
import jax.numpy as jnp
from jax import lax
import jax.experimental.pallas as pl
import jax.experimental.pallas.tpu as pltpu

_HQ, _DH = 32, 192
_LN_EPS = 1e-5
_LANES = 128
_SUB = 8

_COLS = 2048
_ROWS = 24
_SLOTS = 3
_SLAB = 256
_STEP = 512
_Q_STEPS = 16
_F_BLK = 256
_WO_GROUP = 8
_WO_STAGES = (8, 8, 8, 4, 2, 1, 1)


def _silu(v):
    return v * (1.0 / (1.0 + jnp.exp(-v)))


def _loop(n, body, init=None):
    return lax.fori_loop(0, n, body, init)


def _ds(start, size, align):
    return pl.ds(pl.multiple_of(start, align), size)


def _wait_filled(buf, sem):
    pltpu.make_async_copy(buf, buf, sem).wait()


def _start(copies):
    for n, (src, dst, sem) in enumerate(copies):
        pltpu.make_async_copy(src, dst, sem).start(priority=n % 2)


def _kernel(x_hbm, kt_hbm, vt_hbm, wq_hbm, wo_hbm, w1_hbm, w3_hbm, w2_hbm, out_ref,
            x_vm, k_vm, v_vm, wq_vm, wo_vm, w1_vm, w3_vm, w2_vm,
            q_col, o_col, s_vm, y_vm, k_sem, v_sem, w_sem, wo_sem):
    f32, bf16 = jnp.float32, jnp.bfloat16
    d_model = x_vm.shape[1]
    d_ff = w2_vm.shape[0]
    win = k_vm.shape[2]
    win0 = kt_hbm.shape[3] - win
    n_steps = win // _STEP
    n_groups = wo_vm.shape[0]
    row_tiles = _DH // _SUB
    kv_pieces = row_tiles * (win // _COLS) // n_steps
    early = 2 * 2 * kv_pieces

    def start_kv(src, dst, sem, head, j):
        slot = head % _SLOTS
        per_col = row_tiles // kv_pieces
        col = (j // per_col) * _COLS
        rows = _ds((j % per_col) * kv_pieces * _SUB, kv_pieces * _SUB, _SUB)
        src = src.at[0, head, rows, _ds(win0 + col, _COLS, _COLS)]
        dst = dst.at[slot, rows, _ds(col, _COLS, _COLS)]
        _start([(src.at[pl.ds(i * _SUB, _SUB), :], dst.at[pl.ds(i * _SUB, _SUB), :], sem.at[slot])
                for i in range(kv_pieces)])

    def start_head(head):
        _loop(n_steps, lambda j, _: start_kv(kt_hbm, k_vm, k_sem, head, j))
        _loop(n_steps, lambda j, _: start_kv(vt_hbm, v_vm, v_sem, head, j))

    def start_wq(i, _):
        tiles = d_model // _SUB // _Q_STEPS
        n_col = wq_vm.shape[1] // _COLS
        copies = []
        for n in range(tiles * n_col):
            rows = _ds((i + _Q_STEPS * (n % tiles)) * _SUB, _SUB, _SUB)
            cols = pl.ds((n % n_col) * _COLS, _COLS)
            copies.append((wq_hbm.at[rows, cols], wq_vm.at[rows, cols], w_sem.at[0]))
        _start(copies)

    def start_ffn(i):
        copies = []
        for n in range(d_model // _SUB // _Q_STEPS):
            rows = _ds((i + _Q_STEPS * n) * _SUB, _SUB, _SUB)
            copies.append((w1_hbm.at[rows, :], w1_vm.at[rows, :], w_sem.at[1]))
            copies.append((w3_hbm.at[rows, :], w3_vm.at[rows, :], w_sem.at[1]))
            if n < d_ff // _ROWS // _Q_STEPS:
                rows = _ds((i + _Q_STEPS * n) * _ROWS, _ROWS, _SUB)
                copies.append((w2_hbm.at[rows, :], w2_vm.at[rows, :], w_sem.at[1]))
        _start(copies)

    def wo_rows(group, i):
        return _ds((group + n_groups * i) * _ROWS, _ROWS, _SUB)

    def start_wo(group):
        stage, first = 0, 0
        for size in _WO_STAGES[:-1]:
            first += size
            stage = stage + (group >= first).astype(jnp.int32)
        _start([(wo_hbm.at[wo_rows(group, i), :],
                 wo_vm.at[group, pl.ds(i * _ROWS, _ROWS), :], wo_sem.at[stage])
                for i in range(_WO_GROUP)])

    def next_head(phase, head, j):
        src, dst, sem = ((kt_hbm, k_vm, k_sem), (vt_hbm, v_vm, v_sem))[phase]
        start_kv(src, dst, sem, head + 2, j)

    def next_wo(phase, head, j):
        pl.when(j < kv_pieces)(
            lambda: start_wo((2 * (head + 2 - _HQ) + phase) * kv_pieces + j))

    x_copy = pltpu.make_async_copy(x_hbm, x_vm, w_sem.at[0])
    x_copy.start()
    _loop(_Q_STEPS, start_wq)
    start_head(0)
    x_copy.wait()
    _wait_filled(wq_vm, w_sem.at[0])

    x = x_vm[...].astype(f32)
    xc = x - jnp.mean(x, axis=-1, keepdims=True)
    var = jnp.mean(xc * xc, axis=-1, keepdims=True)
    xn = xc / jnp.sqrt(var + _LN_EPS)
    xn8 = jnp.broadcast_to(xn, (_SUB, d_model)).astype(bf16)
    q_blk = wq_vm.shape[1] // _Q_STEPS

    def project_q(i, _):
        start_ffn(i)
        q = jnp.dot(xn8, wq_vm[:, _ds(i * q_blk, q_blk, _LANES)],
                    preferred_element_type=f32) * (_DH ** -0.5)
        for c in range(0, q_blk, _LANES):
            tile = jnp.broadcast_to(q[0:1, c:c + _LANES], (_LANES, _LANES))
            q_col[_ds(i * q_blk + c, _LANES, _LANES), :] = tile.T

    _loop(_Q_STEPS, project_q)
    start_head(1)
    for buf in (w1_vm, w3_vm, w2_vm):
        _wait_filled(buf, w_sem.at[1])
    y_vm[...] = jnp.zeros(y_vm.shape, f32)

    def ffn_block(j):
        cols = _ds(j * _F_BLK, _F_BLK, _F_BLK)
        gate = jnp.dot(xn8, w1_vm[:, cols], preferred_element_type=f32)
        up = jnp.dot(xn8, w3_vm[:, cols], preferred_element_type=f32)
        hidden = (_silu(gate) * up).astype(bf16)
        y_vm[...] += jnp.dot(hidden, w2_vm[cols, :], preferred_element_type=f32)

    def head_step(head, prefetch, with_ffn):
        slot = head % _SLOTS
        head_rows = _ds(head * _DH, _DH, _SUB)
        if with_ffn:
            pl.when(head < d_ff // _F_BLK)(lambda: ffn_block(head))

        _wait_filled(k_vm.at[slot], k_sem.at[slot])
        q = q_col[head_rows, :]
        q = jnp.concatenate([q] * (_SLAB // _LANES), axis=1)

        def scores(j, run_max):
            prefetch(0, head, j)
            for c in range(0, _STEP, _SLAB):
                cols = _ds(j * _STEP + c, _SLAB, _SLAB)
                k = k_vm[slot, :, cols].astype(f32)
                s = jnp.broadcast_to(jnp.sum(k * q, axis=0, keepdims=True), (_SUB, _SLAB))
                s_vm[:, cols] = s
                run_max = jnp.maximum(run_max, s)
            return run_max

        run_max = _loop(n_steps, scores, jnp.full((_SUB, _SLAB), -jnp.inf, f32))
        row_max = jnp.max(run_max, axis=1, keepdims=True)

        _wait_filled(v_vm.at[slot], v_sem.at[slot])

        def values(j, carry):
            acc, total = carry
            prefetch(1, head, j)
            for c in range(0, _STEP, _SLAB):
                cols = _ds(j * _STEP + c, _SLAB, _SLAB)
                p = jnp.exp(s_vm[:, cols] - row_max)
                v = v_vm[slot, :, cols].astype(f32)
                for t in range(0, _SLAB, _LANES):
                    pt = p[:, t:t + _LANES]
                    acc = acc + v[:, t:t + _LANES] * jnp.concatenate([pt] * row_tiles, axis=0)
                    total = total + pt
            return acc, total

        acc, total = _loop(n_steps, values,
                           (jnp.zeros((_DH, _LANES), f32), jnp.zeros((_SUB, _LANES), f32)))
        denom = jnp.sum(total, axis=1, keepdims=True)[0:1, :]
        o = jnp.sum(acc, axis=1, keepdims=True) / denom
        o_col[head_rows, :] = jnp.broadcast_to(o, (_DH, _LANES))

    lax.fori_loop(0, _HQ - 2, lambda h, _: head_step(h, next_head, True), None)
    lax.fori_loop(_HQ - 2, _HQ, lambda h, _: head_step(h, next_wo, False), None)

    g = _silu(y_vm[0:1, :])

    def project_group(group, acc):
        for i in range(_WO_GROUP):
            w = wo_vm[group, i * _ROWS:(i + 1) * _ROWS, :].astype(f32)
            o = jnp.concatenate([o_col[wo_rows(group, i), :]] * (d_model // _LANES), axis=1)
            acc = acc + jnp.sum((w * o).reshape(_ROWS // _SUB, _SUB, d_model), axis=0)
        return acc

    acc = jnp.zeros((_SUB, d_model), f32)
    first = 0
    for stage, size in enumerate(_WO_STAGES):
        def step(t, acc, first=first):
            if first + early < n_groups:
                pl.when(first + t + early < n_groups)(lambda: start_wo(first + t + early))
            return project_group(first + t, acc)

        _wait_filled(wo_vm.at[pl.ds(first, size)], wo_sem.at[stage])
        acc = _loop(size, step, acc)
        first += size
    s = jnp.sum(acc, axis=0, keepdims=True)
    out_ref[...] = (x + s * g).astype(out_ref.dtype)


@jax.jit
def pallas_recurrent_scan__sliding_block_cached__glu_gated_swiglu__decode_kernel(
    A_x: jax.Array,
    A_k_cache: jax.Array,
    A_v_cache: jax.Array,
    A_wq: jax.Array,
    A_wo: jax.Array,
    B_x: jax.Array,
    B_w1: jax.Array,
    B_w3: jax.Array,
    B_w2: jax.Array,
):
    del B_x
    batch, seq, d_model = A_x.shape
    _, n_kv, s_k, d_head = A_k_cache.shape
    assert (batch, seq, n_kv, d_head) == (1, 1, _HQ, _DH)
    win = min(4096, max(256, s_k // 4))
    group_rows = _WO_GROUP * _ROWS

    kt = jnp.swapaxes(A_k_cache, 2, 3)
    vt = jnp.swapaxes(A_v_cache, 2, 3)

    f32 = jnp.float32
    hbm = pl.BlockSpec(memory_space=pltpu.HBM)
    out = pl.pallas_call(
        _kernel,
        out_shape=jax.ShapeDtypeStruct((1, d_model), A_x.dtype),
        in_specs=[hbm] * 8,
        out_specs=pl.BlockSpec(memory_space=pltpu.VMEM),
        scratch_shapes=[
            pltpu.VMEM((1, d_model), A_x.dtype),
            pltpu.VMEM((_SLOTS, _DH, win), kt.dtype),
            pltpu.VMEM((_SLOTS, _DH, win), vt.dtype),
            pltpu.VMEM(A_wq.shape, A_wq.dtype),
            pltpu.VMEM((A_wo.shape[0] // group_rows, group_rows, d_model), A_wo.dtype),
            pltpu.VMEM(B_w1.shape, B_w1.dtype),
            pltpu.VMEM(B_w3.shape, B_w3.dtype),
            pltpu.VMEM(B_w2.shape, B_w2.dtype),
            pltpu.VMEM((_HQ * _DH, _LANES), f32),
            pltpu.VMEM((_HQ * _DH, _LANES), f32),
            pltpu.VMEM((_SUB, win), f32),
            pltpu.VMEM((_SUB, d_model), f32),
            pltpu.SemaphoreType.DMA((_SLOTS,)),
            pltpu.SemaphoreType.DMA((_SLOTS,)),
            pltpu.SemaphoreType.DMA((2,)),
            pltpu.SemaphoreType.DMA((len(_WO_STAGES),)),
        ],
        compiler_params=pltpu.CompilerParams(vmem_limit_bytes=64 * 1024 * 1024),
    )(A_x.reshape(1, d_model), kt, vt, A_wq, A_wo, B_w1, B_w3, B_w2)
    return out.reshape(A_x.shape)
```

```python
import functools

import jax
import jax.numpy as jnp
from jax import lax
import jax.experimental.pallas as pl
import jax.experimental.pallas.tpu as pltpu

_HQ, _DH = 32, 192
_LN_EPS = 1e-5
_LANES = 128
_SUB = 8

_COLS = 2048
_W2_ROWS = 24
_WO_TILES = 16
_BATCH = 6
_W_STRIDE = 20
_SLOTS = 3
_SLAB = 256
_Q_STEPS = 16
_F_BLK = 256


def _silu(v):
    return v * (1.0 / (1.0 + jnp.exp(-v)))


def _loop(lo, hi, body, init=None):
    return lax.fori_loop(lo, hi, body, init)


def _ds(start, size, align):
    return pl.ds(pl.multiple_of(start, align), size)


def _start(copies):
    for n, (src, dst, sem) in enumerate(copies):
        pltpu.make_async_copy(src, dst, sem).start(priority=n % 2)


def _wait_filled(buf, sem):
    pltpu.make_async_copy(buf, buf, sem).wait()


def _stream(x_hbm, kt_hbm, vt_hbm, wq_hbm, wo_hbm, w1_hbm, w3_hbm, w2_hbm, out_ref,
            x_vm, k_vm, v_vm, wq_vm, wo_vm, w1_vm, w3_vm, w2_vm,
            q_col, o_col, s_vm, y_vm, *, k_sem, v_sem, w_sem, wo_sem):
    f32, bf16 = jnp.float32, jnp.bfloat16
    x_sem, wq_sem, w1_sem, w3_sem, w2_sem = (w_sem.at[i] for i in range(5))
    d_model = x_vm.shape[1]
    d_ff = w2_vm.shape[0]
    win = k_vm.shape[2]
    win0 = kt_hbm.shape[3] - win
    row_tiles = _DH // _SUB
    col_tiles = d_model // _LANES
    n_steps = row_tiles * (win // _COLS) // _BATCH
    step = win // n_steps
    n_batches = wo_vm.shape[0]

    def start_kv(src, dst, sem, head, j):
        slot = head % _SLOTS
        per = _BATCH // (win // _COLS)
        half = n_steps // 2
        first = (j % half) * per * 2 + j // half
        copies = []
        for i in range(per):
            rows = _ds((first + 2 * i) * _SUB, _SUB, _SUB)
            for c in range(0, win, _COLS):
                copies.append((src.at[0, head, rows, pl.ds(win0 + c, _COLS)],
                               dst.at[slot, rows, pl.ds(c, _COLS)], sem.at[slot]))
        _start(copies)

    def start_head(head):
        _loop(0, n_steps, lambda j, _: start_kv(kt_hbm, k_vm, k_sem, head, j))
        _loop(0, n_steps, lambda j, _: start_kv(vt_hbm, v_vm, v_sem, head, j))

    def start_wq(j, _):
        n_col = wq_vm.shape[1] // _COLS
        copies = []
        for i in range(d_model // _SUB * n_col // _W_STRIDE):
            piece = j + _W_STRIDE * i
            rows = _ds(lax.div(piece, n_col) * _SUB, _SUB, _SUB)
            cols = _ds(lax.rem(piece, n_col) * _COLS, _COLS, _COLS)
            copies.append((wq_hbm.at[rows, cols], wq_vm.at[rows, cols], wq_sem))
        _start(copies)

    def start_ffn(j, with_w2):
        copies = []
        for i in range(d_model // _SUB // _W_STRIDE):
            rows = _ds((j + _W_STRIDE * i) * _SUB, _SUB, _SUB)
            copies.append((w1_hbm.at[rows, :], w1_vm.at[rows, :], w1_sem))
            copies.append((w3_hbm.at[rows, :], w3_vm.at[rows, :], w3_sem))
            if with_w2:
                rows = _ds((j + _Q_STEPS * i) * _W2_ROWS, _W2_ROWS, _SUB)
                copies.append((w2_hbm.at[rows, :], w2_vm.at[rows, :], w2_sem))
        _start(copies)

    def start_wo(batch):
        _start([(wo_hbm.at[pl.ds((batch + n_batches * i) * _WO_TILES, _WO_TILES)],
                 wo_vm.at[batch, pl.ds(i * _WO_TILES, _WO_TILES)], wo_sem.at[batch])
                for i in range(_BATCH)])

    x_copy = pltpu.make_async_copy(x_hbm, x_vm, x_sem)
    x_copy.start()
    _loop(0, _W_STRIDE, start_wq)
    start_head(0)
    x_copy.wait()
    _wait_filled(wq_vm, wq_sem)

    x = x_vm[...].astype(f32)
    xc = x - jnp.mean(x, axis=-1, keepdims=True)
    var = jnp.mean(xc * xc, axis=-1, keepdims=True)
    xn = xc / jnp.sqrt(var + _LN_EPS)
    xn8 = jnp.broadcast_to(xn, (_SUB, d_model)).astype(bf16)
    q_blk = wq_vm.shape[1] // _Q_STEPS

    def project_q(i, _):
        start_ffn(i, True)
        q = jnp.dot(xn8, wq_vm[:, _ds(i * q_blk, q_blk, _LANES)],
                    preferred_element_type=f32) * (_DH ** -0.5)
        for c in range(0, q_blk, _LANES):
            tile = jnp.broadcast_to(q[0:1, c:c + _LANES], (_LANES, _LANES))
            q_col[_ds(i * q_blk + c, _LANES, _LANES), :] = tile.T

    _loop(0, _Q_STEPS, project_q)
    _loop(_Q_STEPS, _W_STRIDE, lambda j, _: start_ffn(j, False))
    start_head(1)
    _wait_filled(w1_vm, w1_sem)
    _wait_filled(w3_vm, w3_sem)
    _wait_filled(w2_vm, w2_sem)
    y_vm[...] = jnp.zeros(y_vm.shape, f32)

    def ffn_block(j):
        cols = _ds(j * _F_BLK, _F_BLK, _F_BLK)
        gate = jnp.dot(xn8, w1_vm[:, cols], preferred_element_type=f32)
        up = jnp.dot(xn8, w3_vm[:, cols], preferred_element_type=f32)
        hidden = (_silu(gate) * up).astype(bf16)
        y_vm[...] += jnp.dot(hidden, w2_vm[cols, :], preferred_element_type=f32)

    def attend(head, prefetch):
        slot = head % _SLOTS
        head_rows = _ds(head * _DH, _DH, _SUB)

        _wait_filled(k_vm.at[slot], k_sem.at[slot])
        q = q_col[head_rows, :]
        q = jnp.concatenate([q] * (_SLAB // _LANES), axis=1)

        def scores(j, run_max):
            prefetch(0, j)
            for c in range(0, step, _SLAB):
                cols = _ds(j * step + c, _SLAB, _SLAB)
                k = k_vm[slot, :, cols].astype(f32)
                s = jnp.broadcast_to(jnp.sum(k * q, axis=0, keepdims=True), (_SUB, _SLAB))
                s_vm[:, cols] = s
                run_max = jnp.maximum(run_max, s)
            return run_max

        run_max = _loop(0, n_steps, scores, jnp.full((_SUB, _SLAB), -jnp.inf, f32))
        row_max = jnp.max(run_max, axis=1, keepdims=True)

        _wait_filled(v_vm.at[slot], v_sem.at[slot])

        def values(j, carry):
            acc, total = carry
            prefetch(1, j)
            for c in range(0, step, _SLAB):
                cols = _ds(j * step + c, _SLAB, _SLAB)
                p = jnp.exp(s_vm[:, cols] - row_max)
                v = v_vm[slot, :, cols].astype(f32)
                for t in range(0, _SLAB, _LANES):
                    pt = p[:, t:t + _LANES]
                    acc = acc + v[:, t:t + _LANES] * jnp.concatenate([pt] * row_tiles, axis=0)
                    total = total + pt
            return acc, total

        acc, total = _loop(0, n_steps, values,
                           (jnp.zeros((_DH, _LANES), f32), jnp.zeros((_SUB, _LANES), f32)))
        denom = jnp.sum(total, axis=1, keepdims=True)[0:1, :]
        o = jnp.sum(acc, axis=1, keepdims=True) / denom
        o_col[head_rows, :] = jnp.broadcast_to(o, (_DH, _LANES))

    def early_head(head, _):
        pl.when(head < d_ff // _F_BLK)(lambda: ffn_block(head))
        caches = ((kt_hbm, k_vm, k_sem), (vt_hbm, v_vm, v_sem))
        attend(head, lambda phase, j: start_kv(*caches[phase], head + 2, j))

    def late_head(head, _):
        done = (head - (_HQ - 2)) * 2 * n_steps
        attend(head, lambda phase, j: start_wo(done + phase * n_steps + j))

    _loop(0, _HQ - 2, early_head)
    _loop(_HQ - 2, _HQ, late_head)

    g = _silu(y_vm[0:1, :])
    started = 2 * 2 * n_steps

    def project_out(u, acc):
        acc = list(acc)
        for phase in range(col_tiles):
            batch = u * col_tiles + phase
            pl.when(batch + started < n_batches)(lambda: start_wo(batch + started))
            _wait_filled(wo_vm.at[batch], wo_sem.at[batch])
            for i in range(_BATCH):
                w = wo_vm[batch, i * _WO_TILES:(i + 1) * _WO_TILES].astype(f32)
                block0 = (u + n_batches // col_tiles * i) * _WO_TILES
                for t in range(_WO_TILES):
                    block, col = divmod(phase * _WO_TILES + t, col_tiles)
                    o = o_col[_ds((block0 + block) * _SUB, _SUB, _SUB), :]
                    acc[col] = acc[col] + w[t] * o
        return tuple(acc)

    acc = _loop(0, n_batches // col_tiles, project_out,
                (jnp.zeros((_SUB, _LANES), f32),) * col_tiles)
    s = jnp.sum(jnp.concatenate(acc, axis=1), axis=0, keepdims=True)
    out_ref[...] = (x + s * g).astype(out_ref.dtype)


def _kernel(*refs, n_batches):
    dma = pltpu.SemaphoreType.DMA
    pl.run_scoped(functools.partial(_stream, *refs),
                  k_sem=dma((_SLOTS,)), v_sem=dma((_SLOTS,)), w_sem=dma((5,)),
                  wo_sem=dma((n_batches,)))


@jax.jit
def pallas_recurrent_scan__sliding_block_cached__glu_gated_swiglu__decode_kernel(
    A_x: jax.Array,
    A_k_cache: jax.Array,
    A_v_cache: jax.Array,
    A_wq: jax.Array,
    A_wo: jax.Array,
    B_x: jax.Array,
    B_w1: jax.Array,
    B_w3: jax.Array,
    B_w2: jax.Array,
):
    del B_x
    d_model = A_x.shape[-1]
    assert A_x.shape == (1, 1, 640) and B_w2.shape == (1536, 640)
    assert A_k_cache.shape[:2] == (1, _HQ) and A_k_cache.shape[3] == _DH
    win = min(4096, max(256, A_k_cache.shape[2] // 4))
    assert win == 4096

    kt = jnp.swapaxes(A_k_cache, 2, 3)
    vt = jnp.swapaxes(A_v_cache, 2, 3)
    wo_tiles = (A_wo.reshape(-1, _SUB, d_model // _LANES, _LANES)
                .transpose(0, 2, 1, 3).reshape(-1, _SUB, _LANES))
    n_batches = wo_tiles.shape[0] // (_BATCH * _WO_TILES)

    f32 = jnp.float32
    out = pl.pallas_call(
        functools.partial(_kernel, n_batches=n_batches),
        out_shape=jax.ShapeDtypeStruct((1, d_model), A_x.dtype),
        in_specs=[pl.BlockSpec(memory_space=pltpu.HBM)] * 8,
        out_specs=pl.BlockSpec(memory_space=pltpu.VMEM),
        scratch_shapes=[
            pltpu.VMEM((1, d_model), A_x.dtype),
            pltpu.VMEM((_SLOTS, _DH, win), kt.dtype),
            pltpu.VMEM((_SLOTS, _DH, win), vt.dtype),
            pltpu.VMEM(A_wq.shape, A_wq.dtype),
            pltpu.VMEM((n_batches, _BATCH * _WO_TILES, _SUB, _LANES), A_wo.dtype),
            pltpu.VMEM(B_w1.shape, B_w1.dtype),
            pltpu.VMEM(B_w3.shape, B_w3.dtype),
            pltpu.VMEM(B_w2.shape, B_w2.dtype),
            pltpu.VMEM((_HQ * _DH, _LANES), f32),
            pltpu.VMEM((_HQ * _DH, _LANES), f32),
            pltpu.VMEM((_SUB, win), f32),
            pltpu.VMEM((_SUB, d_model), f32),
        ],
        compiler_params=pltpu.CompilerParams(vmem_limit_bytes=64 * 1024 * 1024),
    )(A_x.reshape(1, d_model), kt, vt, A_wq, wo_tiles, B_w1, B_w3, B_w2)
    return out.reshape(A_x.shape)
```

```python
import functools

import jax
import jax.numpy as jnp
from jax import lax
import jax.experimental.pallas as pl
import jax.experimental.pallas.tpu as pltpu

_HQ, _DH = 32, 192
_LN_EPS = 1e-5
_LANES = 128
_SUB = 8

_COLS = 2048
_W2_ROWS = 24
_WO_TILES = 16
_BATCH = 6
_W_STRIDE = 20
_SLOTS = 3
_SLAB = 256
_Q_STEPS = 16
_F_BLK = 256


def _silu(v):
    return v * (1.0 / (1.0 + jnp.exp(-v)))


def _loop(lo, hi, body, init=None):
    return lax.fori_loop(lo, hi, body, init)


def _ds(start, size, align):
    return pl.ds(pl.multiple_of(start, align), size)


def _start(copies):
    for n, (src, dst, sem) in enumerate(copies):
        pltpu.make_async_copy(src, dst, sem).start(priority=n % 2)


def _wait_filled(buf, sem):
    pltpu.make_async_copy(buf, buf, sem).wait()


def _stream(x_hbm, kt_hbm, vt_hbm, wq_hbm, wo_hbm, w1_hbm, w3_hbm, w2_hbm, out_ref,
            x_vm, k_vm, v_vm, wq_vm, wo_vm, w1_vm, w3_vm, w2_vm,
            q_col, o_col, s_vm, y_vm, *, k_sem, v_sem, w_sem, wo_sem):
    f32, bf16 = jnp.float32, jnp.bfloat16
    x_sem, wq_sem, w1_sem, w3_sem, w2_sem = (w_sem.at[i] for i in range(5))
    d_model = x_vm.shape[1]
    d_ff = w2_vm.shape[0]
    win = k_vm.shape[2]
    win0 = kt_hbm.shape[3] - win
    row_tiles = _DH // _SUB
    col_tiles = d_model // _LANES
    n_steps = row_tiles * (win // _COLS) // _BATCH
    step = win // n_steps
    n_batches = wo_vm.shape[0]
    pairs = _BATCH // 2

    def start_kv(src, dst, sem, head, j):
        slot = head % _SLOTS
        per = _BATCH // (win // _COLS)
        half = n_steps // 2
        first = (j % half) * per * 2 + j // half
        copies = []
        for i in range(per):
            rows = _ds((first + 2 * i) * _SUB, _SUB, _SUB)
            for c in range(0, win, _COLS):
                copies.append((src.at[0, head, rows, pl.ds(win0 + c, _COLS)],
                               dst.at[slot, rows, pl.ds(c, _COLS)], sem.at[slot]))
        _start(copies)

    def start_head(head):
        _loop(0, n_steps, lambda j, _: start_kv(kt_hbm, k_vm, k_sem, head, j))
        _loop(0, n_steps, lambda j, _: start_kv(vt_hbm, v_vm, v_sem, head, j))

    def start_wq():
        n_col = wq_vm.shape[1] // _COLS
        n_pieces = d_model // _SUB * n_col
        copies = []
        for j in range(_W_STRIDE):
            for piece in range(j, n_pieces, _W_STRIDE):
                window = (pl.ds(piece // n_col * _SUB, _SUB), pl.ds(piece % n_col * _COLS, _COLS))
                copies.append((wq_hbm.at[window], wq_vm.at[window], wq_sem))
        _start(copies)

    def start_ffn(j, with_w2):
        copies = []
        for i in range(d_model // _SUB // _W_STRIDE):
            rows = _ds((j + _W_STRIDE * i) * _SUB, _SUB, _SUB)
            copies.append((w1_hbm.at[rows, :], w1_vm.at[rows, :], w1_sem))
            copies.append((w3_hbm.at[rows, :], w3_vm.at[rows, :], w3_sem))
            if with_w2:
                rows = _ds((j + _Q_STEPS * i) * _W2_ROWS, _W2_ROWS, _SUB)
                copies.append((w2_hbm.at[rows, :], w2_vm.at[rows, :], w2_sem))
        _start(copies)

    def start_wo(batch):
        _start([(wo_hbm.at[pl.ds((batch + n_batches * i) * _WO_TILES, _WO_TILES)],
                 wo_vm.at[batch, pl.ds(i * _WO_TILES, _WO_TILES)], wo_sem.at[batch * pairs + i // 2])
                for i in range(_BATCH)])

    x_copy = pltpu.make_async_copy(x_hbm, x_vm, x_sem)
    x_copy.start()
    start_wq()
    start_head(0)
    x_copy.wait()
    _wait_filled(wq_vm, wq_sem)

    x = x_vm[...].astype(f32)
    xc = x - jnp.mean(x, axis=-1, keepdims=True)
    var = jnp.mean(xc * xc, axis=-1, keepdims=True)
    xn = xc / jnp.sqrt(var + _LN_EPS)
    xn8 = jnp.broadcast_to(xn, (_SUB, d_model)).astype(bf16)
    q_blk = wq_vm.shape[1] // _Q_STEPS

    def project_q(i, _):
        start_ffn(i, True)
        q = jnp.dot(xn8, wq_vm[:, _ds(i * q_blk, q_blk, _LANES)],
                    preferred_element_type=f32) * (_DH ** -0.5)
        for c in range(0, q_blk, _LANES):
            tile = jnp.broadcast_to(q[0:1, c:c + _LANES], (_LANES, _LANES))
            q_col[_ds(i * q_blk + c, _LANES, _LANES), :] = tile.T

    _loop(0, _Q_STEPS, project_q)
    _loop(_Q_STEPS, _W_STRIDE, lambda j, _: start_ffn(j, False))
    start_head(1)
    _wait_filled(w1_vm, w1_sem)
    _wait_filled(w3_vm, w3_sem)
    _wait_filled(w2_vm, w2_sem)
    y_vm[...] = jnp.zeros(y_vm.shape, f32)

    def ffn_block(j):
        cols = _ds(j * _F_BLK, _F_BLK, _F_BLK)
        gate = jnp.dot(xn8, w1_vm[:, cols], preferred_element_type=f32)
        up = jnp.dot(xn8, w3_vm[:, cols], preferred_element_type=f32)
        hidden = (_silu(gate) * up).astype(bf16)
        y_vm[...] += jnp.dot(hidden, w2_vm[cols, :], preferred_element_type=f32)

    def attend(head, prefetch):
        slot = head % _SLOTS
        head_rows = _ds(head * _DH, _DH, _SUB)

        _wait_filled(k_vm.at[slot], k_sem.at[slot])
        q = q_col[head_rows, :]
        q = jnp.concatenate([q] * (_SLAB // _LANES), axis=1)

        def scores(j, run_max):
            prefetch(0, j)
            for c in range(0, step, _SLAB):
                cols = _ds(j * step + c, _SLAB, _SLAB)
                k = k_vm[slot, :, cols].astype(f32)
                s = jnp.broadcast_to(jnp.sum(k * q, axis=0, keepdims=True), (_SUB, _SLAB))
                s_vm[:, cols] = s
                run_max = jnp.maximum(run_max, s)
            return run_max

        run_max = _loop(0, n_steps, scores, jnp.full((_SUB, _SLAB), -jnp.inf, f32))
        row_max = jnp.max(run_max, axis=1, keepdims=True)

        _wait_filled(v_vm.at[slot], v_sem.at[slot])

        def values(j, carry):
            acc, total = carry
            prefetch(1, j)
            for c in range(0, step, _SLAB):
                cols = _ds(j * step + c, _SLAB, _SLAB)
                p = jnp.exp(s_vm[:, cols] - row_max)
                v = v_vm[slot, :, cols].astype(f32)
                for t in range(0, _SLAB, _LANES):
                    pt = p[:, t:t + _LANES]
                    acc = acc + v[:, t:t + _LANES] * jnp.concatenate([pt] * row_tiles, axis=0)
                    total = total + pt
            return acc, total

        acc, total = _loop(0, n_steps, values,
                           (jnp.zeros((_DH, _LANES), f32), jnp.zeros((_SUB, _LANES), f32)))
        denom = jnp.sum(total, axis=1, keepdims=True)[0:1, :]
        o = jnp.sum(acc, axis=1, keepdims=True) / denom
        o_col[head_rows, :] = jnp.broadcast_to(o, (_DH, _LANES))

    def early_head(head, _):
        pl.when(head < d_ff // _F_BLK)(lambda: ffn_block(head))
        caches = ((kt_hbm, k_vm, k_sem), (vt_hbm, v_vm, v_sem))
        attend(head, lambda phase, j: start_kv(*caches[phase], head + 2, j))

    def late_head(head, _):
        done = (head - (_HQ - 2)) * 2 * n_steps
        attend(head, lambda phase, j: start_wo(done + phase * n_steps + j))

    _loop(0, _HQ - 2, early_head)
    _loop(_HQ - 2, _HQ, late_head)

    g = _silu(y_vm[0:1, :])
    started = 2 * 2 * n_steps

    def project_out(u, acc):
        acc = list(acc)
        for phase in range(col_tiles):
            batch = u * col_tiles + phase
            pl.when(batch + started < n_batches)(lambda: start_wo(batch + started))
            for i in range(_BATCH):
                if i % 2 == 0:
                    _wait_filled(wo_vm.at[batch, pl.ds(i * _WO_TILES, 2 * _WO_TILES)],
                                 wo_sem.at[batch * pairs + i // 2])
                w = wo_vm[batch, i * _WO_TILES:(i + 1) * _WO_TILES].astype(f32)
                block0 = (u + n_batches // col_tiles * i) * _WO_TILES
                for t in range(_WO_TILES):
                    block, col = divmod(phase * _WO_TILES + t, col_tiles)
                    o = o_col[_ds((block0 + block) * _SUB, _SUB, _SUB), :]
                    acc[col] = acc[col] + w[t] * o
        return tuple(acc)

    acc = _loop(0, n_batches // col_tiles, project_out,
                (jnp.zeros((_SUB, _LANES), f32),) * col_tiles)
    s = jnp.sum(jnp.concatenate(acc, axis=1), axis=0, keepdims=True)
    out_ref[...] = (x + s * g).astype(out_ref.dtype)


def _kernel(*refs, n_batches):
    dma = pltpu.SemaphoreType.DMA
    pl.run_scoped(functools.partial(_stream, *refs),
                  k_sem=dma((_SLOTS,)), v_sem=dma((_SLOTS,)), w_sem=dma((5,)),
                  wo_sem=dma((n_batches * _BATCH // 2,)))


@jax.jit
def pallas_recurrent_scan__sliding_block_cached__glu_gated_swiglu__decode_kernel(
    A_x: jax.Array,
    A_k_cache: jax.Array,
    A_v_cache: jax.Array,
    A_wq: jax.Array,
    A_wo: jax.Array,
    B_x: jax.Array,
    B_w1: jax.Array,
    B_w3: jax.Array,
    B_w2: jax.Array,
):
    del B_x
    d_model = A_x.shape[-1]
    assert A_x.shape == (1, 1, 640) and B_w2.shape == (1536, 640)
    assert A_k_cache.shape[:2] == (1, _HQ) and A_k_cache.shape[3] == _DH
    win = min(4096, max(256, A_k_cache.shape[2] // 4))
    assert win == 4096

    kt = jnp.swapaxes(A_k_cache, 2, 3)
    vt = jnp.swapaxes(A_v_cache, 2, 3)
    wo_tiles = (A_wo.reshape(-1, _SUB, d_model // _LANES, _LANES)
                .transpose(0, 2, 1, 3).reshape(-1, _SUB, _LANES))
    n_batches = wo_tiles.shape[0] // (_BATCH * _WO_TILES)

    f32 = jnp.float32
    out = pl.pallas_call(
        functools.partial(_kernel, n_batches=n_batches),
        out_shape=jax.ShapeDtypeStruct((1, d_model), A_x.dtype),
        in_specs=[pl.BlockSpec(memory_space=pltpu.HBM)] * 8,
        out_specs=pl.BlockSpec(memory_space=pltpu.VMEM),
        scratch_shapes=[
            pltpu.VMEM((1, d_model), A_x.dtype),
            pltpu.VMEM((_SLOTS, _DH, win), kt.dtype),
            pltpu.VMEM((_SLOTS, _DH, win), vt.dtype),
            pltpu.VMEM(A_wq.shape, A_wq.dtype),
            pltpu.VMEM((n_batches, _BATCH * _WO_TILES, _SUB, _LANES), A_wo.dtype),
            pltpu.VMEM(B_w1.shape, B_w1.dtype),
            pltpu.VMEM(B_w3.shape, B_w3.dtype),
            pltpu.VMEM(B_w2.shape, B_w2.dtype),
            pltpu.VMEM((_HQ * _DH, _LANES), f32),
            pltpu.VMEM((_HQ * _DH, _LANES), f32),
            pltpu.VMEM((_SUB, win), f32),
            pltpu.VMEM((_SUB, d_model), f32),
        ],
        compiler_params=pltpu.CompilerParams(vmem_limit_bytes=64 * 1024 * 1024),
    )(A_x.reshape(1, d_model), kt, vt, A_wq, wo_tiles, B_w1, B_w3, B_w2)
    return out.reshape(A_x.shape)
```
